```python
import os as _os
_os.environ.setdefault("JAX_PLATFORMS", "cpu")
import jax
import jax.numpy as jnp

def _softmax(x, axis=-1):
    return jax.nn.softmax(x, axis=axis)
def _gelu(x):
    return jax.nn.gelu(x, approximate=True)
def _silu(x):
    return jax.nn.silu(x)
def _sigmoid(x):
    return jax.nn.sigmoid(x)
def _layernorm(x, axis=-1, eps=1e-5):
    m = jnp.mean(x, axis=axis, keepdims=True)
    v = jnp.var(x, axis=axis, keepdims=True)
    return (x - m) / jnp.sqrt(v + eps)
def _scatter_add(tgt, idx, src, axis=0):
    return tgt.at[idx].add(src)
def _segment_sum(src, seg, n):
    return jax.ops.segment_sum(src, seg, n)
class _Rng:
    def __init__(self, key):
        self._k = key
    def _next(self):
        self._k, sub = jax.random.split(self._k)
        return sub
    def normal(self, shape):
        return jax.random.normal(self._next(), shape, dtype=jnp.bfloat16)
    def randint(self, lo, hi, shape):
        return jax.random.randint(self._next(), shape, lo, hi, dtype=jnp.int32)
    def uniform(self, shape, lo=0.0, hi=1.0):
        return jax.random.uniform(self._next(), shape, jnp.bfloat16, lo, hi)
    def permutation(self, n):
        return jax.random.permutation(self._next(), n)


kernel_name = 'concat_heads__gqa_block_cached__mha_block_cached__near_ridge'

def setup_inputs():
    _rng = _Rng(jax.random.key(int.from_bytes(__import__("os").urandom(4), "little")))
    _w = (lambda a: (lambda t: t.astype(jnp.bfloat16) if jnp.issubdtype(t.dtype, jnp.floating) else t)(jnp.asarray(a)))
    def _A_setup():
        B, Sq, D = 8, 48, 512
        Hq, Hkv, Sk, Dh = 32, 8, 1024, 128
        assert Hq % Hkv == 0, (Hq, Hkv)
        return {
            "x": _w((lambda *s: _rng.normal(s) * 0.8)(B, Sq, D)),
            "k_cache": _w((lambda *s: _rng.normal(s) * 0.8)(B, Hkv, Sk, Dh)),
            "v_cache": _w((lambda *s: _rng.normal(s) * 0.05)(B, Hkv, Sk, Dh)),
            "wq": _w((lambda *s: _rng.normal(s) * 0.8)(D, Hq * Dh) * (D ** -0.5)),
            "wo": _w((lambda *s: _rng.normal(s) * 0.05)(Hq * Dh, D) * ((Hq * Dh) ** -0.5)),
        }
    _A_in = _A_setup()

    def _B_setup():
        B, Sq, D = 8, 48, 512
        H, Sk, Dh = 32, 1024, 128
        return {
            "x": _w((lambda *s: _rng.normal(s) * 0.8)(B, Sq, D)),
            "k_cache": _w((lambda *s: _rng.normal(s) * 0.8)(B, H, Sk, Dh)),
            "v_cache": _w((lambda *s: _rng.normal(s) * 0.05)(B, H, Sk, Dh)),
            "wq": _w((lambda *s: _rng.normal(s) * 0.8)(D, H * Dh) * (D ** -0.5)),
            "wo": _w((lambda *s: _rng.normal(s) * 0.05)(H * Dh, D) * ((H * Dh) ** -0.5)),
        }
    _B_in = _B_setup()

    return {
        "A_x": _A_in["x"],
        "A_k_cache": _A_in["k_cache"],
        "A_v_cache": _A_in["v_cache"],
        "A_wq": _A_in["wq"],
        "A_wo": _A_in["wo"],
        "B_x": _B_in["x"],
        "B_k_cache": _B_in["k_cache"],
        "B_v_cache": _B_in["v_cache"],
        "B_wq": _B_in["wq"],
        "B_wo": _B_in["wo"],
    }

def reference(A_x, A_k_cache, A_v_cache, A_wq, A_wo, B_x, B_k_cache, B_v_cache, B_wq, B_wo):
    def _A_ref(x, k_cache, v_cache, wq, wo):
        B, Sq, D = x.shape
        Hq, Dh = 32, 128
        Hkv = k_cache.shape[1]
        rep = Hq // Hkv
        q = (lambda x, *d: x.transpose(*d))((x @ wq).reshape(B, Sq, Hq, Dh), 0, 2, 1, 3)
        k = jnp.repeat(k_cache, rep, axis=1)
        v = jnp.repeat(v_cache, rep, axis=1)
        scores = jnp.einsum("bhqd,bhkd->bhqk", q, k) * (Dh ** -0.5)
        p = _softmax(scores, axis=-1)
        o = jnp.einsum("bhqk,bhkd->bhqd", p, v)
        return (lambda x, *d: x.transpose(*d))(o, 0, 2, 1, 3).reshape(B, Sq, Hq * Dh) @ wo

    def _B_ref(x, k_cache, v_cache, wq, wo):
        B, Sq, D = x.shape
        H, Dh = 32, 128
        q = (lambda x, *d: x.transpose(*d))((x @ wq).reshape(B, Sq, H, Dh), 0, 2, 1, 3)
        scores = jnp.einsum("bhqd,bhkd->bhqk", q, k_cache) * (Dh ** -0.5)
        p = _softmax(scores, axis=-1)
        o = jnp.einsum("bhqk,bhkd->bhqd", p, v_cache)
        return (lambda x, *d: x.transpose(*d))(o, 0, 2, 1, 3).reshape(B, Sq, H * Dh) @ wo

    a = _A_ref(A_x, A_k_cache, A_v_cache, A_wq, A_wo)
    b = _B_ref(B_x, B_k_cache, B_v_cache, B_wq, B_wo)
    return jnp.concatenate([a, b], axis=-1)
```

```python
import functools
import math

import jax
import jax.numpy as jnp
from jax import lax
from jax.experimental import pallas as pl
from jax.experimental.pallas import tpu as pltpu

NB, SQ, D = 8, 48, 512
HQ, HKV, SK, DH = 32, 8, 1024, 128
REP = HQ // HKV
M = NB * SQ
PIECE = 128
WPIECE = 32
NT = (((1,), (1,)), ((), ()))
QSCALE = DH ** -0.5 * math.log2(math.e)
BF, F32 = jnp.bfloat16, jnp.float32


def build(UA=2, UB=4, do_compute=True, do_dma=True, nosem=False, flags=None):
    def kernel(ax, ak, av, awq, awo, bx, bk, bv, bwq, bwo, out,
               x_v, wq_v, woa_v, wob_v, ka_v, va_v, kb_v, vb_v,
               qa_v, qb_v, pa_v, la_v, pb_v, lb_v, oa_v, ob_v, acc_a, acc_b, out_v,
               sem_x, sem_w, sem_ka, sem_va, sem_kb, sem_vb, sem_o):

        def kv_descs(src, h, dst, sem):
            def start(j, b):
                if not do_dma:
                    return
                r = j * PIECE
                if not isinstance(r, int):
                    r = pl.multiple_of(r, PIECE)
                pltpu.make_async_copy(src.at[b, h, pl.ds(r, PIECE)], dst.at[b, pl.ds(r, PIECE)], sem).start(priority=b % 2)
            return start

        def w_descs(g):
            c = g * (REP * DH)
            if not isinstance(c, int):
                c = pl.multiple_of(c, REP * DH)
            slot = g % 2

            def start(j, b):
                if not do_dma:
                    return
                r = (2 * j + b // 4) * WPIECE
                if not isinstance(r, int):
                    r = pl.multiple_of(r, WPIECE)
                m = b % 4
                if m == 0:
                    s, d = awq.at[pl.ds(r, WPIECE), pl.ds(c, REP * DH)], wq_v.at[0, pl.ds(r, WPIECE)]
                elif m == 1:
                    s, d = bwq.at[pl.ds(r, WPIECE), pl.ds(c, REP * DH)], wq_v.at[1, pl.ds(r, WPIECE)]
                elif m == 2:
                    s, d = awo.at[pl.ds(c + r, WPIECE)], woa_v.at[pl.ds(r, WPIECE)]
                else:
                    s, d = bwo.at[pl.ds(c + r, WPIECE)], wob_v.at[slot, pl.ds(r, WPIECE)]
                pltpu.make_async_copy(s, d, sem_w).start(priority=b % 2)
            return start

        def wait_all(ref, sem):
            if do_dma:
                pltpu.make_async_copy(ref, ref, sem).wait()

        def issue(start, j):
            for b in range(NB):
                start(j, b)

        def qk_task(q_v, k_ref, p_v, l_v, U, start):
            def body(i, _):
                for u in range(U):
                    b = i * U + u
                    issue(start, b)
                    if do_compute:
                        s = lax.dot_general(q_v(b), k_ref[b], NT, preferred_element_type=F32)
                        m = jnp.max(s, axis=-1, keepdims=True)
                        p = jnp.exp2(s - m)
                        p_v[b] = p.astype(BF)
                        l_v[b] = jnp.broadcast_to(jnp.sum(p, axis=-1, keepdims=True), l_v.shape[1:])
            lax.fori_loop(0, NB // U, body, None)

        def pv_task(v_ref, p_v, l_v, store, U, start):
            def body(i, _):
                for u in range(U):
                    b = i * U + u
                    issue(start, b)
                    if do_compute:
                        o = jnp.dot(p_v[b], v_ref[b], preferred_element_type=F32)
                        store(b, (o / l_v[b]).astype(BF))
            lax.fori_loop(0, NB // U, body, None)

        def rows(b):
            r = b * SQ
            return pl.ds(r if isinstance(r, int) else pl.multiple_of(r, 16), SQ)

        def store_a(b, o):
            for j in range(REP):
                oa_v[rows(b), j * DH:(j + 1) * DH] = o[j * SQ:(j + 1) * SQ]

        def store_b(j):
            def f(b, o):
                ob_v[j, rows(b), :] = o
            return f

        def q_proj(start):
            issue(start, 0); issue(start, 1)
            if do_compute:
                q = jnp.dot(x_v[0], wq_v[0], preferred_element_type=F32) * QSCALE
                q = q.astype(BF)
                for b in range(NB):
                    for j in range(REP):
                        qa_v[b, j * SQ:(j + 1) * SQ, :] = q[b * SQ:(b + 1) * SQ, j * DH:(j + 1) * DH]
            issue(start, 2); issue(start, 3); issue(start, 4); issue(start, 5)
            if do_compute:
                q = jnp.dot(x_v[1], wq_v[1], preferred_element_type=F32) * QSCALE
                q = q.astype(BF)
                for j in range(REP):
                    qb_v[j] = q[:, j * DH:(j + 1) * DH]
            issue(start, 6); issue(start, 7)

        def o_proj_a():
            if do_compute:
                acc_a[...] += jnp.dot(oa_v[...], woa_v[...], preferred_element_type=F32)

        def o_proj_b(slot):
            if do_compute:
                o = jnp.concatenate([ob_v[j] for j in range(REP)], axis=1)
                acc_b[...] += jnp.dot(o, wob_v[slot], preferred_element_type=F32)

        nothing = lambda j, b: None

        def b_qk(j, start):
            wait_all(kb_v.at[j], sem_kb.at[j])
            qk_task(lambda b: qb_v[j, rows(b), :], kb_v.at[j], pb_v, lb_v, UB, start)

        def b_pv(j, start):
            wait_all(vb_v.at[j], sem_vb.at[j])
            pv_task(vb_v.at[j], pb_v, lb_v, store_b(j), UB, start)

        if do_dma:
            for i in range(M // WPIECE):
                r = pl.ds(i * WPIECE, WPIECE)
                pltpu.make_async_copy(ax.at[r], x_v.at[0, r], sem_x).start(priority=0)
                pltpu.make_async_copy(bx.at[r], x_v.at[1, r], sem_x).start(priority=1)
        for start in (w_descs(0), kv_descs(ak, 0, ka_v, sem_ka)):
            lax.fori_loop(0, NB, lambda j, _, start=start: issue(start, j), None)
        acc_a[...] = jnp.zeros_like(acc_a)
        acc_b[...] = jnp.zeros_like(acc_b)
        wait_all(x_v, sem_x)

        def step(g, _):
            @pl.when(g > 0)
            def _():
                b_qk(REP - 1, w_descs(g))
                b_pv(REP - 1, kv_descs(ak, g, ka_v, sem_ka))
                o_proj_b((g - 1) % 2)

            wait_all(ka_v, sem_w)
            q_proj(kv_descs(av, g, va_v, sem_va))

            wait_all(ka_v, sem_ka)
            qk_task(lambda b: qa_v[b], ka_v, pa_v, la_v, UA, kv_descs(bk, g * REP, kb_v.at[0], sem_kb.at[0]))
            wait_all(va_v, sem_va)
            pv_task(va_v, pa_v, la_v, store_a, UA, kv_descs(bv, g * REP, vb_v.at[0], sem_vb.at[0]))

            def head(j, _):
                b_qk(j, kv_descs(bk, g * REP + j + 1, kb_v.at[j + 1], sem_kb.at[j + 1]))

                @pl.when(j == 0)
                def _():
                    o_proj_a()
                b_pv(j, kv_descs(bv, g * REP + j + 1, vb_v.at[j + 1], sem_vb.at[j + 1]))
            lax.fori_loop(0, REP - 1, head, None)

        lax.fori_loop(0, HKV, step, None)

        out_v[0] = acc_a[...].astype(BF)
        cpa = pltpu.make_async_copy(out_v.at[0], out.at[:, pl.ds(0, D)], sem_o.at[0])
        cpa.start()
        b_qk(REP - 1, nothing)
        b_pv(REP - 1, nothing)
        o_proj_b((HKV - 1) % 2)
        out_v[1] = acc_b[...].astype(BF)
        cpb = pltpu.make_async_copy(out_v.at[1], out.at[:, pl.ds(D, D)], sem_o.at[1])
        cpb.start()
        cpa.wait()
        cpb.wait()

    VM = pltpu.VMEM
    DMA = pltpu.SemaphoreType.DMA
    scratch = [
        VM((2, M, D), BF),
        VM((2, D, REP * DH), BF),
        VM((REP * DH, D), BF),
        VM((2, REP * DH, D), BF),
        VM((NB, SK, DH), BF),
        VM((NB, SK, DH), BF),
        VM((REP, NB, SK, DH), BF),
        VM((REP, NB, SK, DH), BF),
        VM((NB, REP * SQ, DH), BF),
        VM((REP, M, DH), BF),
        VM((NB, REP * SQ, SK), BF),
        VM((NB, REP * SQ, DH), F32),
        VM((NB, SQ, SK), BF),
        VM((NB, SQ, DH), F32),
        VM((M, REP * DH), BF),
        VM((REP, M, DH), BF),
        VM((M, D), F32),
        VM((M, D), F32),
        VM((2, M, D), BF),
        DMA, DMA, DMA, DMA, DMA((REP,)), DMA((REP,)), DMA((2,)),
    ]

    @jax.jit
    def fn(A_x, A_k_cache, A_v_cache, A_wq, A_wo, B_x, B_k_cache, B_v_cache, B_wq, B_wo):
        out = pl.pallas_call(
            kernel,
            out_shape=jax.ShapeDtypeStruct((M, 2 * D), BF),
            in_specs=[pl.BlockSpec(memory_space=pl.ANY)] * 10,
            out_specs=pl.BlockSpec(memory_space=pl.ANY),
            scratch_shapes=scratch,
            compiler_params=pltpu.CompilerParams(
                vmem_limit_bytes=100 * 2**20, disable_bounds_checks=True,
                disable_semaphore_checks=nosem, flags=flags),
        )(A_x.reshape(M, D), A_k_cache, A_v_cache, A_wq, A_wo,
          B_x.reshape(M, D), B_k_cache, B_v_cache, B_wq, B_wo)
        return out.reshape(NB, SQ, 2 * D)

    return fn


_fn = build()


@jax.jit
def pallas_concat_heads__gqa_block_cached__mha_block_cached__near_ridge_kernel(
    A_x, A_k_cache, A_v_cache, A_wq, A_wo, B_x, B_k_cache, B_v_cache, B_wq, B_wo
):
    return _fn(A_x, A_k_cache, A_v_cache, A_wq, A_wo, B_x, B_k_cache, B_v_cache, B_wq, B_wo)
```

```python
import functools
import math

import jax
import jax.numpy as jnp
from jax import lax
from jax.experimental import pallas as pl
from jax.experimental.pallas import tpu as pltpu

NB, SQ, D = 8, 48, 512
HQ, HKV, SK, DH = 32, 8, 1024, 128
REP = HQ // HKV
M = NB * SQ
GW = REP * DH
NT = (((1,), (1,)), ((), ()))
QSCALE = DH ** -0.5 * math.log2(math.e)
BF, F32 = jnp.bfloat16, jnp.float32
KA, VA, KB, VB = 0, 1, 2, 2 + REP


def _aligned(i, n):
    return i if isinstance(i, int) else pl.multiple_of(i, n)


def build(do_compute=True, do_dma=True, nosem=False, flags=None,
          pat="pair", apat=None, wpat="slab", tail_groups=((0, 4), (4, 2), (6, 1), (7, 1)), bitcast=False,
          outprio=0, off="", last_a=(3, 3, 2, 0), apos=0, tpat=None):
    apat = apat or pat
    tpat = tpat or pat

    def kernel(ax, ak, av, awq, awo, bx, bk, bv, bwq, bwo, out,
               x_v, w_v, kv_v, q_v, pa_v, la_v, pb_v, lb_v, o_v, acc_v, out_v,
               sem_w, sem_kv, sem_t, sem_o):

        def copy(s, d, sem, prio):
            if do_dma:
                pltpu.make_async_copy(s, d, sem).start(priority=prio)

        def wait_all(ref, sem):
            if do_dma:
                pltpu.make_async_copy(ref, ref, sem).wait()

        def wait_kv(slot):
            wait_all(kv_v.at[slot], sem_kv.at[slot])

        def kv_ticks(src, h, slot):
            p = apat if src is ak or src is av else pat
            dst, sem = kv_v.at[slot], sem_kv.at[slot]

            def tick(t):
                if p == "contig":
                    r = pl.ds(_aligned(t * 128, 128), 128)
                    for b in range(NB):
                        copy(src.at[b, h, r], dst.at[b, r], sem, b % 2)
                elif p == "pair":
                    for s in range(2):
                        r = pl.ds(_aligned(t * 128 + s * 64, 64), 64)
                        for i, b in enumerate((0, 4, 2, 6)):
                            bb = pl.ds(b, 2)
                            copy(src.at[bb, h, r], dst.at[bb, r], sem, i % 2)
            return tick

        def tail_ticks(src, h, slot):
            dst = kv_v.at[slot]
            descs = []
            for gi, (b0, nb) in enumerate(tail_groups):
                if nb == 1:
                    for j in range(8):
                        jj = (j // 2) + 4 * (j % 2)
                        descs.append((pl.ds(b0, 1), pl.ds(jj * 128, 128), gi))
                elif tpat == "pair":
                    for s in range(16):
                        for b in range(b0, b0 + nb, 2):
                            descs.append((pl.ds(b, 2), pl.ds(s * 64 if nb > 2 else (s // 2 + 8 * (s % 2)) * 64, 64), gi))
                else:
                    for s in range(8):
                        for b in range(b0, b0 + nb):
                            descs.append((pl.ds(b, 1), pl.ds(s * 128 if nb > 2 else (s // 2 + 4 * (s % 2)) * 128, 128), gi))
            assert len(descs) == 64

            def tick(t):
                for i in range(t * 8, t * 8 + 8):
                    bb, r, gi = descs[i]
                    copy(src.at[bb, h, r], dst.at[bb, r], sem_t.at[gi], i % 2)
            return tick

        def wq_ticks(g):
            c = pl.ds(_aligned(g * GW, GW), GW)

            def tick(t):
                for s in range(4):
                    r = pl.ds(_aligned((4 * t + s) * 32, 32), 32)
                    copy(awq.at[r, c], w_v.at[0, r], sem_w, 0)
                    copy(bwq.at[r, c], w_v.at[1, r], sem_w, 1)
            return tick

        def wo_ticks(g):
            def tick(t):
                for s in range(4):
                    r0 = _aligned(t * 32 + s * 128, 32)
                    r = pl.ds(_aligned(g * GW + r0, 32), 32)
                    copy(awo.at[r], w_v.at[2, pl.ds(r0, 32)], sem_w, 0)
                    copy(bwo.at[r], w_v.at[3, pl.ds(r0, 32)], sem_w, 1)
            return tick

        def w_ticks(g):
            c = pl.ds(_aligned(g * GW, GW), GW)

            def tick(t):
                for s in range(2):
                    r0 = _aligned((2 * t + s) * 32, 32)
                    r = pl.ds(r0, 32)
                    ro = pl.ds(_aligned((g - 1) * GW + r0, 32), 32)
                    copy(awq.at[r, c], w_v.at[0, r], sem_w, 0)
                    copy(bwq.at[r, c], w_v.at[1, r], sem_w, 1)
                    copy(awo.at[ro], w_v.at[2, r], sem_w, 0)
                    copy(bwo.at[ro], w_v.at[3, r], sem_w, 1)
            return tick

        nothing = lambda t: None

        def load_kv(slot, b):
            if bitcast:
                return pltpu.bitcast(kv_v.bitcast(jnp.uint32)[slot, b], BF)
            return kv_v[slot, b]

        def rows(b, n=1):
            return pl.ds(_aligned(b * SQ, 16), n * SQ)

        def softmax_unit(q, k, p_ref, l_ref, i):
            s = lax.dot_general(q, k, NT, preferred_element_type=F32)
            p = jnp.exp2(s - jnp.max(s, axis=-1, keepdims=True))
            p_ref[i] = p.astype(BF)
            l_ref[i] = jnp.broadcast_to(1.0 / jnp.sum(p, axis=-1, keepdims=True), l_ref.shape[1:])

        def pv_unit(v, p_ref, l_ref, i):
            return (jnp.dot(p_ref[i], v, preferred_element_type=F32) * l_ref[i]).astype(BF)

        def a_qk(b, i):
            if do_compute and "aqk" not in off:
                q = jnp.concatenate([q_v[0, j, rows(b), :] for j in range(REP)], axis=0)
                softmax_unit(q, load_kv(KA, b), pa_v, la_v, i)

        def a_pv(b, i):
            if do_compute and "apv" not in off:
                o = pv_unit(load_kv(VA, b), pa_v, la_v, i)
                for j in range(REP):
                    o_v[0, j, rows(b), :] = o[j * SQ:(j + 1) * SQ]

        def b_qk(j, b):
            if do_compute and "bqk" not in off:
                softmax_unit(q_v[1, j, rows(b), :], load_kv(KB + j, b), pb_v, lb_v, b)

        def b_pv(j, b):
            if do_compute and "bpv" not in off:
                o_v[1, j, rows(b), :] = pv_unit(load_kv(VB + j, b), pb_v, lb_v, b)

        def attn_task(b_unit, a_unit, j, tick):
            def body(i, _):
                for u in range(4):
                    tick(4 * i + u)
                    if u == apos:
                        a_unit(2 * j + i, i)
                    b_unit(j, 4 * i + u)
            lax.fori_loop(0, 2, body, None)

        def attn_task_static(b_unit, a_unit, j, ticks, a0, na):
            for b in range(NB):
                for f in ticks[b]:
                    f()
                if b % 2 == 0 and b // 2 < na:
                    a_unit(a0 + b // 2, b // 2)
                b_unit(j, b)

        def q_proj(br, r):
            if do_compute and "qp" not in off:
                q = jnp.dot(x_v[br, r, :], w_v[br], preferred_element_type=F32)
                q = (q * QSCALE).astype(BF)
                for j in range(REP):
                    q_v[br, j, r, :] = q[:, j * DH:(j + 1) * DH]

        def o_proj(br, r, j0=0, j1=REP):
            if do_compute and "op" not in off:
                o = jnp.concatenate([o_v[br, j, r, :] for j in range(j0, j1)], axis=1)
                acc_v[br, r, :] += jnp.dot(o, w_v[2 + br, j0 * DH:j1 * DH, :], preferred_element_type=F32)

        def proj_task(g, t, tick):
            r = pl.ds(t * 128, 128)

            def body(br, _):
                tick(4 * br)
                tick(4 * br + 1)
                if isinstance(g, int):
                    if g > 0:
                        o_proj(br, r)
                else:
                    pl.when(g > 0)(lambda: o_proj(br, r))
                tick(4 * br + 2)
                tick(4 * br + 3)
                q_proj(br, r)
            lax.fori_loop(0, 2, body, None)

        wq0 = wq_ticks(0)
        for t in range(4):
            if t < 3:
                for s in range(4):
                    r = pl.ds((4 * t + s) * 32, 32)
                    copy(ax.at[r], x_v.at[0, r], sem_w, 0)
                    copy(bx.at[r], x_v.at[1, r], sem_w, 1)
            wq0(t)
        ka0 = kv_ticks(ak, 0, KA)
        lax.fori_loop(0, 8, lambda t, _: ka0(t), None)
        acc_v[...] = jnp.zeros_like(acc_v)
        wait_all(x_v, sem_w)
        wait_all(w_v.at[pl.ds(0, 2)], sem_w)

        def proj_tasks(g):
            proj_task(g, 0, kv_ticks(av, g, VA))
            proj_task(g, 1, kv_ticks(bk, g * REP, KB))
            proj_task(g, 2, kv_ticks(bv, g * REP, VB))
            wait_kv(KA)

        def step(g, _):
            proj_tasks(g)

            def head(j, _):
                wait_kv(KB + j)
                attn_task(b_qk, a_qk, j, kv_ticks(bk, g * REP + j + 1, KB + j + 1))

                @pl.when(j == 0)
                def _():
                    wait_kv(VA)
                wait_kv(VB + j)
                attn_task(b_pv, a_pv, j, kv_ticks(bv, g * REP + j + 1, VB + j + 1))
            lax.fori_loop(0, REP - 1, head, None)

            j = REP - 1
            wait_kv(KB + j)
            attn_task(b_qk, a_qk, j, w_ticks(g + 1))
            wait_kv(VB + j)
            attn_task(b_pv, a_pv, j, kv_ticks(ak, g + 1, KA))
            wait_all(w_v, sem_w)

        lax.fori_loop(0, HKV - 1, step, None)

        g = HKV - 1
        proj_tasks(g)
        a0 = [sum(last_a[:j]) for j in range(REP)]
        one = lambda tick: [[functools.partial(tick, t)] for t in range(8)]
        wo = wo_ticks(g)

        wait_kv(KB)
        attn_task_static(b_qk, a_qk, 0, one(kv_ticks(bk, g * REP + 1, KB + 1)), a0[0], last_a[0])
        wait_kv(VA)
        wait_kv(VB)
        tk = one(kv_ticks(bv, g * REP + 1, VB + 1))
        for t in range(4):
            tk[2 * t].append(functools.partial(wo, t))
        attn_task_static(b_pv, a_pv, 0, tk, a0[0], last_a[0])
        wait_kv(KB + 1)
        attn_task_static(b_qk, a_qk, 1, one(kv_ticks(bk, g * REP + 2, KB + 2)), a0[1], last_a[1])
        wait_kv(VB + 1)
        attn_task_static(b_pv, a_pv, 1, one(kv_ticks(bv, g * REP + 2, VB + 2)), a0[1], last_a[1])
        wait_all(w_v.at[pl.ds(2, 2)], sem_w)
        o_proj(1, pl.ds(0, M), 0, 2)
        wait_kv(KB + 2)
        attn_task_static(b_qk, a_qk, 2, one(kv_ticks(bk, g * REP + 3, KB + 3)), a0[2], last_a[2])
        wait_kv(VB + 2)
        tail = tail_ticks(bv, HQ - 1, VB + 3)
        tk = [[functools.partial(tail, b // 2)] if b % 2 == 0 else [] for b in range(NB)]
        attn_task_static(b_pv, a_pv, 2, tk, a0[2], last_a[2])

        @pl.loop(0, 2)
        def _(i):
            @pl.when(i == 0)
            def _():
                tail(4)
                tail(5)

            @pl.when(i == 1)
            def _():
                tail(6)
                tail(7)
            r = pl.ds(pl.multiple_of(i * (M // 2), 16), M // 2)
            o_proj(0, r)
            o_proj(1, r, 2, 3)
            out_v[0, r, :] = acc_v[0, r, :].astype(BF)
            for s in range(6):
                rr = pl.ds(pl.multiple_of(i * (M // 2) + s * 32, 16), 32)
                pltpu.make_async_copy(out_v.at[0, rr], out.at[rr, pl.ds(0, D)], sem_o.at[0]).start(priority=s % 2)

        wait_kv(KB + 3)
        lax.fori_loop(0, 2, lambda i, _: [b_qk(3, 4 * i + u) for u in range(4)] and None, None)
        for gi, (b0, nb) in enumerate(tail_groups):
            wait_all(kv_v.at[VB + 3, pl.ds(b0, nb)], sem_t.at[gi])
            if do_compute and "tail" not in off:
                o = [pv_unit(load_kv(VB + 3, b), pb_v, lb_v, b) for b in range(b0, b0 + nb)]
                o = jnp.concatenate(o, axis=0) if nb > 1 else o[0]
                r = rows(b0, nb)
                y = acc_v[1, r, :] + jnp.dot(o, w_v[3, (REP - 1) * DH:, :], preferred_element_type=F32)
                out_v[1, r, :] = y.astype(BF)
            for b in range(b0, b0 + nb):
                pltpu.make_async_copy(out_v.at[1, rows(b)], out.at[rows(b), pl.ds(D, D)], sem_o.at[1]).start(
                    priority=(b % 2) if outprio == "alt" else outprio)
        pltpu.make_async_copy(out_v.at[0], out_v.at[0], sem_o.at[0]).wait()
        pltpu.make_async_copy(out_v.at[1], out_v.at[1], sem_o.at[1]).wait()

    VM = pltpu.VMEM
    DMA = pltpu.SemaphoreType.DMA
    scratch = [
        VM((2, M, D), BF),
        VM((4, D, GW), BF),
        VM((2 + 2 * REP, NB, SK, DH), BF),
        VM((2, REP, M, DH), BF),
        VM((4, REP * SQ, SK), BF),
        VM((4, REP * SQ, DH), F32),
        VM((NB, SQ, SK), BF),
        VM((NB, SQ, DH), F32),
        VM((2, REP, M, DH), BF),
        VM((2, M, D), F32),
        VM((2, M, D), BF),
        DMA, DMA((2 + 2 * REP,)), DMA((len(tail_groups),)), DMA((2,)),
    ]

    @jax.jit
    def fn(A_x, A_k_cache, A_v_cache, A_wq, A_wo, B_x, B_k_cache, B_v_cache, B_wq, B_wo):
        out = pl.pallas_call(
            kernel,
            out_shape=jax.ShapeDtypeStruct((M, 2 * D), BF),
            in_specs=[pl.BlockSpec(memory_space=pl.ANY)] * 10,
            out_specs=pl.BlockSpec(memory_space=pl.ANY),
            scratch_shapes=scratch,
            compiler_params=pltpu.CompilerParams(
                vmem_limit_bytes=100 * 2**20, disable_bounds_checks=True,
                disable_semaphore_checks=nosem, flags=flags),
        )(A_x.reshape(M, D), A_k_cache, A_v_cache, A_wq, A_wo,
          B_x.reshape(M, D), B_k_cache, B_v_cache, B_wq, B_wo)
        return out.reshape(NB, SQ, 2 * D)

    return fn


_fn = build(pat='contig')


@jax.jit
def pallas_concat_heads__gqa_block_cached__mha_block_cached__near_ridge_kernel(
    A_x, A_k_cache, A_v_cache, A_wq, A_wo, B_x, B_k_cache, B_v_cache, B_wq, B_wo
):
    return _fn(A_x, A_k_cache, A_v_cache, A_wq, A_wo, B_x, B_k_cache, B_v_cache, B_wq, B_wo)
```

```python
import contextlib
import functools
import math

import jax
import jax.numpy as jnp
from jax import lax
from jax.experimental import pallas as pl
from jax.experimental.pallas import tpu as pltpu

NB, SQ, D = 8, 48, 512
HQ, HKV, SK, DH = 32, 8, 1024, 128
REP = HQ // HKV
M = NB * SQ
GW = REP * DH
NA = NB // REP
NU = NB + NA
NT = (((1,), (1,)), ((), ()))
QSCALE = DH ** -0.5 * math.log2(math.e)
BF, F32 = jnp.bfloat16, jnp.float32
S_X, S_WQ, S_WO, S_KV, S_OUT, NSEM = 0, 1, 2, 4, 8, 9

PAIR_EVO = ("2.0 6.0 2.2 6.3 A0 A1 2.1 6.1 0.1 6.2 0.0 4.1 0.2 4.2 A2 A3 2.3 4.0 0.3 4.3 W W", {4: 15, 6: 7}, True)
PAIR_BASE = ("0.0 4.0 2.0 6.0 A0 A1 0.1 4.1 2.1 6.1 0.2 4.2 2.2 6.2 A2 A3 0.3 4.3 2.3 6.3 W W", {}, True)
CONTIG = ("0.0 1.0 2.0 3.0 4.0 5.0 6.0 7.0 A0 A1 0.1 1.1 2.1 3.1 4.1 5.1 6.1 7.1 A2 A3 W W", {}, False)
PATS = dict(evo=PAIR_EVO, base=PAIR_BASE, contig=CONTIG)


def _aligned(i, n):
    return i if isinstance(i, int) else pl.multiple_of(i, n)


def _when(cond, fn):
    if isinstance(cond, bool):
        if cond:
            fn()
    else:
        pl.when(cond)(fn)


def _interleave(a, b):
    out, k = [], 0
    for i in range(0, len(a), 2):
        out += a[i:i + 2]
        while k < len(b) and k * len(a) < (i + 2) * len(b):
            out += b[k:k + 2]
            k += 2
    return out


def build(do_compute=True, do_dma=True, nosem=False, flags=None, off="", pat="contig",
          tail_groups=(4, 4), scopes=False, apos=2, nobc=True, awr="end", cuts=(72, 84, 100, 116)):
    layout, skew, pair = PATS[pat] if isinstance(pat, str) else pat
    layout = layout.split()
    scope = (lambda n: jax.named_scope(n)) if scopes else (lambda n: contextlib.nullcontext())

    def kernel(ax, ak, av, awq, awo, bx, bk, bv, bwq, bwo, out,
               x_v, wq_v, wo_v, kv_v, q_v, pa_v, la_v, pb_v, lb_v, o_v, acc_v, out_v, sems):

        def copy(s, d, sem, p):
            if do_dma:
                pltpu.make_async_copy(s, d, sems.at[sem]).start(priority=p)

        def wait_all(ref, sem):
            if do_dma:
                pltpu.make_async_copy(ref, ref, sems.at[sem]).wait()

        def slot_of(s, is_v):
            return 2 * (s % 2) + is_v

        def gcols(g):
            return pl.ds(_aligned(g * GW, GW), GW)

        def wq_desc(br, half, i, sem, p):
            r, c = pl.ds(_aligned(i * 8, 8), 8), pl.ds(half * 2048, 2048)
            copy((awq, bwq)[br].at[r, c], wq_v.at[br, r, c], sem, p)

        def wo_desc(br, m, p):
            r = pl.ds(_aligned(m * 32, 32), 32)
            copy((awo, bwo)[br].at[r], wo_v.at[br, r], S_WO + (m // 16) % 2, p)

        def x_desc(br, i, p):
            r = pl.ds(i * 32, 32)
            copy((ax, bx)[br].at[r], x_v.at[br, r], S_X, p)

        def b_desc(s, is_v, b, nb, r0, p):
            sl = slot_of(s, is_v)
            r = pl.ds(_aligned(r0, 128 // nb), 128 // nb)
            copy((bk, bv)[is_v].at[pl.ds(b, nb), s, r], kv_v.at[sl, pl.ds(b, nb), r], S_KV + sl, p)

        def a_desc(a, is_v, i, nb, r0, sl, sem, p):
            r = pl.ds(_aligned(r0, 128 // nb), 128 // nb)
            copy((ak, av)[is_v].at[pl.ds(NA * (a % REP) + i, nb), a // REP, r], kv_v.at[sl, pl.ds(NB + i, nb), r], sem, p)

        def quad(s, is_v, i, w=None):
            sl = slot_of(s, is_v)
            seq, wi = [], 0
            for e in layout:
                if e == "W":
                    if w is not None:
                        seq.append(functools.partial(w, wi))
                    wi += 1
                elif e[0] == "A":
                    t = int(e[1])
                    if pair:
                        n = 4 * i + t
                        args = (0, 2, ((n + skew[8]) % 16 if 8 in skew else n) * 64)
                    else:
                        n = 2 * i + t // 2
                        args = (t % 2, 1, ((n + skew[8 + t % 2]) % 8 if 8 + t % 2 in skew else n) * 128)
                    f = functools.partial(a_desc, s + 1, is_v, *args, sl, S_KV + sl)
                    seq.append(lambda p, f=f: _when(s + 1 < HQ, lambda: f(p)))
                else:
                    b, t = (int(z) for z in e.split("."))
                    if pair:
                        n = 4 * i + t
                        seq.append(functools.partial(b_desc, s, is_v, b, 2, ((n + skew[b]) % 16 if b in skew else n) * 64))
                    else:
                        n = 2 * i + t
                        seq.append(functools.partial(b_desc, s, is_v, b, 1, ((n + skew[b]) % 8 if b in skew else n) * 128))
            return seq

        def issue(seq, lo, hi):
            for n in range(lo, min(hi, len(seq))):
                seq[n](n % 2)

        def rows(b, n=1):
            return pl.ds(_aligned(b * SQ, 16), n * SQ)

        def arows(a):
            return rows(NA * (a % REP), NA)

        def softmax_unit(q, k, p_ref, l_ref, i):
            s = lax.dot_general(q, k, NT, preferred_element_type=F32)
            p = jnp.exp2(s - jnp.max(s, axis=-1, keepdims=True))
            p_ref[i] = p.astype(BF)
            l_ref[i] = jnp.broadcast_to(1.0 / jnp.sum(p, axis=-1, keepdims=True), l_ref.shape[1:])

        def pv_unit(v, p_ref, l_ref, i):
            return (jnp.dot(p_ref[i], v, preferred_element_type=F32) * l_ref[i]).astype(BF)

        def a_qk(sl, i):
            if do_compute and "aqk" not in off:
                softmax_unit(q_v[0, rows(REP * i, REP), :], kv_v[sl, NB + i], pa_v, la_v, i)

        def a_pv(sl, i):
            if do_compute and "apv" not in off:
                o_v[0, rows(REP * i, REP), :] = pv_unit(kv_v[sl, NB + i], pa_v, la_v, i)

        def b_qk(sl, b):
            if do_compute and "bqk" not in off:
                softmax_unit(q_v[1, rows(b), :], kv_v[sl, b], pb_v, lb_v, b)

        def b_pv(sl, b):
            if do_compute and "bpv" not in off:
                o_v[1, rows(b), :] = pv_unit(kv_v[sl, b], pb_v, lb_v, b)

        def q_proj_a(a):
            if do_compute and "qp" not in off:
                q = jnp.dot(x_v[0, arows(a), :], wq_v[0, :, gcols(a // REP)], preferred_element_type=F32)
                q = (q * QSCALE).astype(BF)
                for i in range(NA):
                    for j in range(REP):
                        q_v[0, rows(REP * i + j), :] = q[i * SQ:(i + 1) * SQ, j * DH:(j + 1) * DH]

        def q_proj_b(s):
            if do_compute and "qp" not in off:
                c = pl.ds(_aligned(s * DH, DH), DH)
                q = jnp.dot(x_v[1], wq_v[1, :, c], preferred_element_type=F32)
                q_v[1] = (q * QSCALE).astype(BF)

        def o_proj_a(a):
            if do_compute and "op" not in off:
                o = jnp.concatenate(
                    [jnp.concatenate([o_v[0, rows(REP * i + j), :] for j in range(REP)], axis=1) for i in range(NA)],
                    axis=0)
                acc_v[0, arows(a), :] += jnp.dot(o, wo_v[0, gcols(a // REP), :], preferred_element_type=F32)

        def o_proj_b(s):
            if do_compute and "op" not in off:
                r = pl.ds(_aligned(s * DH, DH), DH)
                acc_v[1] += jnp.dot(o_v[1], wo_v[1, r, :], preferred_element_type=F32)

        def phase(b_unit, a_unit, sl, seq_of):
            def body(i, _):
                seq = seq_of(i)
                per = -(-len(seq) // 4)
                per += per % 2
                for u in range(4):
                    issue(seq, u * per, (u + 1) * per)
                    if u == apos and a_unit is not None:
                        a_unit(sl, i)
                    b_unit(sl, 4 * i + u)
            lax.fori_loop(0, 2, body, None)

        def step(s, _):
            def wq_w(i):
                return lambda br, p: _when(s < 14, lambda: wq_desc(br, 1, 8 + 4 * s + i, S_WQ, p))

            def wo_w(i):
                return lambda br, p: _when(s < 27, lambda: wo_desc(br, 20 + 4 * s + i, p))

            with scope("step"):
                sl = slot_of(s, 0)
                wait_all(kv_v.at[sl], S_KV + sl)
                phase(b_qk, a_qk, sl, lambda i: quad(s + 1, 0, 2 * i, wq_w(2 * i)) + quad(s + 1, 0, 2 * i + 1, wq_w(2 * i + 1)))
                _when(s == 14, lambda: wait_all(wq_v.at[:, :, pl.ds(2048, 2048)], S_WQ))
                q_proj_a(jnp.minimum(s + 2, HQ - 1))
                q_proj_b(s + 1)
                sl = slot_of(s, 1)
                wait_all(kv_v.at[sl], S_KV + sl)
                phase(b_pv, a_pv, sl, lambda i: quad(s + 1, 1, 2 * i, wo_w(2 * i)) + quad(s + 1, 1, 2 * i + 1, wo_w(2 * i + 1)))
                g = (s + 1) // REP
                _when((s + 1) % REP == 0, lambda: wait_all(wo_v.at[:, gcols(g), :], S_WO + g % 2))
                o_proj_a(s + 1)
                o_proj_b(s)

        with scope("prologue"):
            part = functools.partial
            kv = [d for i in range(4) for d in quad(0, 0, i)]
            if pair:
                kv += [part(a_desc, 0, v, 0, 2, t * 64, 2 + v, S_X) for t in range(16) for v in range(2)]
            else:
                kv += [part(a_desc, 0, v, i, 1, t * 128, 2 + v, S_X) for t in range(8) for v in range(2) for i in range(2)]
            w = [part(x_desc, br, i) for i in range(12) for br in range(2)]
            w += [part(wq_desc, br, 0, (i // 8) + 8 * (i % 8), S_X) for i in range(64) for br in range(2)]
            seq = _interleave(w, kv)
            issue(seq, 0, len(seq))
            acc_v[...] = jnp.zeros_like(acc_v)
            w = [part(wo_desc, br, m) for m in range(20) for br in range(2)]
            w += [part(wq_desc, br, 1, i, S_WQ) for i in range(8) for br in range(2)]
            seq = _interleave(w, [d for i in range(4) for d in quad(0, 1, i)])
            issue(seq, 0, cuts[0])
            wait_all(x_v, S_X)
            wait_all(wq_v.at[:, :, pl.ds(0, 2048)], S_X)
            wait_all(kv_v.at[pl.ds(2, 2), pl.ds(NB, NA)], S_X)
            q_proj_a(0)
            issue(seq, cuts[0], cuts[1])
            a_qk(2, 0)
            a_qk(2, 1)
            issue(seq, cuts[1], cuts[2])
            a_pv(3, 0)
            a_pv(3, 1)
            issue(seq, cuts[2], cuts[3])
            q_proj_b(0)
            q_proj_a(1)
            issue(seq, cuts[3], len(seq))
            wait_all(wo_v.at[:, gcols(0), :], S_WO)
            o_proj_a(0)

        lax.fori_loop(0, HQ - 1, step, None)

        with scope("tail"):
            s = HQ - 1

            def write(br, b):
                r, c = rows(b), pl.ds(br * D, D)
                pltpu.make_async_copy(out_v.at[r, c], out.at[r, c], sems.at[S_OUT]).start(priority=b % 2)

            out_v[:, 0:D] = acc_v[0].astype(BF)
            if awr == "end":
                for b in range(NB):
                    write(0, b)
            sl = slot_of(s, 0)
            wait_all(kv_v.at[sl, pl.ds(0, NB)], S_KV + sl)
            phase(b_qk, None, sl, lambda i: [])
            sl = slot_of(s, 1)
            wait_all(kv_v.at[sl, pl.ds(0, NB)], S_KV + sl)
            if awr == "late":
                for b in range(NB):
                    write(0, b)
            b0 = 0
            for nb in tail_groups:
                if do_compute and "tail" not in off:
                    o = [pv_unit(kv_v[sl, b], pb_v, lb_v, b) for b in range(b0, b0 + nb)]
                    o = jnp.concatenate(o, axis=0) if nb > 1 else o[0]
                    r = rows(b0, nb)
                    y = acc_v[1, r, :] + jnp.dot(o, wo_v[1, s * DH:(s + 1) * DH, :], preferred_element_type=F32)
                    out_v[r, D:2 * D] = y.astype(BF)
                for b in range(b0, b0 + nb):
                    write(1, b)
                b0 += nb
            pltpu.make_async_copy(out_v, out_v, sems.at[S_OUT]).wait()

    VM = pltpu.VMEM
    scratch = [
        VM((2, M, D), BF),
        VM((2, D, HQ * DH), BF),
        VM((2, HQ * DH, D), BF),
        VM((4, NU, SK, DH), BF),
        VM((2, M, DH), BF),
        VM((NA, REP * SQ, SK), BF),
        VM((NA, REP * SQ, DH), F32),
        VM((NB, SQ, SK), BF),
        VM((NB, SQ, DH), F32),
        VM((2, M, DH), BF),
        VM((2, M, D), F32),
        VM((M, 2 * D), BF),
        pltpu.SemaphoreType.DMA((NSEM,)),
    ]

    @jax.jit
    def fn(A_x, A_k_cache, A_v_cache, A_wq, A_wo, B_x, B_k_cache, B_v_cache, B_wq, B_wo):
        out = pl.pallas_call(
            kernel,
            out_shape=jax.ShapeDtypeStruct((M, 2 * D), BF),
            in_specs=[pl.BlockSpec(memory_space=pl.ANY)] * 10,
            out_specs=pl.BlockSpec(memory_space=pl.ANY),
            scratch_shapes=scratch,
            compiler_params=pltpu.CompilerParams(
                vmem_limit_bytes=100 * 2**20, disable_bounds_checks=nobc,
                disable_semaphore_checks=nosem, flags=flags),
        )(A_x.reshape(M, D), A_k_cache, A_v_cache, A_wq, A_wo,
          B_x.reshape(M, D), B_k_cache, B_v_cache, B_wq, B_wo)
        return out.reshape(NB, SQ, 2 * D)

    return fn


_fn = build(awr='late')


@jax.jit
def pallas_concat_heads__gqa_block_cached__mha_block_cached__near_ridge_kernel(
    A_x, A_k_cache, A_v_cache, A_wq, A_wo, B_x, B_k_cache, B_v_cache, B_wq, B_wo
):
    return _fn(A_x, A_k_cache, A_v_cache, A_wq, A_wo, B_x, B_k_cache, B_v_cache, B_wq, B_wo)
```

```python
import contextlib
import functools
import math

import jax
import jax.numpy as jnp
from jax import lax
from jax.experimental import pallas as pl
from jax.experimental.pallas import tpu as pltpu

NB, SQ, D = 8, 48, 512
HQ, HKV, SK, DH = 32, 8, 1024, 128
REP = HQ // HKV
M = NB * SQ
GW = REP * DH
NA = NB // REP
NU = NB + NA
NT = (((1,), (1,)), ((), ()))
QSCALE = DH ** -0.5 * math.log2(math.e)
BF, F32 = jnp.bfloat16, jnp.float32

CONTIG = "0.0 1.0 2.0 3.0 4.0 5.0 6.0 7.0 A0 A1 0.1 1.1 2.1 3.1 4.1 5.1 6.1 7.1 A2 A3 W W"


def _aligned(i, n):
    return i if isinstance(i, int) else pl.multiple_of(i, n)


def _mod(i, n):
    return i % n if isinstance(i, int) else jnp.bitwise_and(i, n - 1)


def _div(i, n):
    return i // n if isinstance(i, int) else lax.shift_right_logical(i, n.bit_length() - 1)


def _when(cond, fn):
    if isinstance(cond, bool):
        if cond:
            fn()
    else:
        pl.when(cond)(fn)


def _interleave(a, b):
    out, k = [], 0
    for i in range(0, len(a), 2):
        out += a[i:i + 2]
        while k < len(b) and k * len(a) < (i + 2) * len(b):
            out += b[k:k + 2]
            k += 2
    return out


def build(do_compute=True, do_dma=True, nosem=True, flags=None, off="", layout=CONTIG,
          scopes=False, apos=0, ppos=1, nobc=True, cuts=(72, 84, 100, 116),
          wqo=1, woo=0, pro=3, late=1, wfirst="late", split=0, hold_at=0, spread=None, nslot=2, wp=('alt', 'alt', 'alt'), big=False, warm=0, warm2=0):
    toks = layout.split()
    scope = (lambda n: jax.named_scope(n)) if scopes else (lambda n: contextlib.nullcontext())
    S_X, S_A0, S_WQ, S_WO, S_OUT, S_T, S_KV = 0, 1, 2, 4, 6, 7, 9
    NSEM = S_KV + 4

    def slab(b):
        return (b % 2) * (NB // 2) + b // 2

    def kernel(ax, ak, av, awq, awo, bx, bk, bv, bwq, bwo, out,
               x_v, wq_v, wo_v, kv_v, q_v, pa_v, la_v, pb_v, lb_v, o_v, acc_v, out_v, sems):

        def copy(s, d, sem, p):
            if do_dma:
                pltpu.make_async_copy(s, d, sems.at[sem]).start(priority=p)

        def wait_all(ref, sem):
            if do_dma:
                pltpu.make_async_copy(ref, ref, sems.at[sem]).wait()

        def slot_of(s, is_v):
            return 2 * _mod(s, 2) + is_v

        def gcols(g):
            return pl.ds(_aligned(g * GW, GW), GW)

        def wq_desc(br, half, i, p):
            r, c = pl.ds(_aligned(i * 8, 8), 8), pl.ds(half * 2048, 2048)
            copy((awq, bwq)[br].at[r, c], wq_v.at[br, r, c], S_WQ + half, p)

        def wo_desc(br, m, p):
            r = pl.ds(_aligned(m * 32, 32), 32)
            copy((awo, bwo)[br].at[r], wo_v.at[br, r], S_WO + _mod(_div(m, 16), 2), p)

        def x_desc(br, i, p):
            r = pl.ds(i * 32, 32)
            copy((ax, bx)[br].at[r], x_v.at[br, r], S_X, p)

        def b_desc(s, is_v, b, piece, sem, p):
            r = pl.ds(piece * 128, 128)
            copy((bk, bv)[is_v].at[b, s, r], kv_v.at[slot_of(s, is_v), slab(b), r], sem, p)

        def a_desc(a, is_v, i, piece, sl, sem, p):
            r = pl.ds(piece * 128, 128)
            copy((ak, av)[is_v].at[NA * _mod(a, REP) + i, _div(a, REP), r], kv_v.at[sl, NB + i, r], sem, p)

        def quad(s, is_v, i, w=None):
            sl = slot_of(s, is_v)
            sem = S_KV + sl
            seq, wi = [], 0
            for e in toks:
                if e == "W":
                    if w is not None:
                        seq.append(functools.partial(w, wi))
                    wi += 1
                elif e[0] == "A":
                    t = int(e[1])
                    f = functools.partial(a_desc, s + 1, is_v, t % 2, 2 * i + t // 2, sl, sem)
                    seq.append(lambda p, f=f: _when(s + 1 < HQ, lambda: f(p)))
                else:
                    b, t = (int(z) for z in e.split("."))
                    assert b % 2 == len(seq) % 2
                    if is_v and b % 2 == 0:
                        f = functools.partial(b_desc, s, is_v, b, 2 * i + t, sem)
                        seq.append(lambda p, f=f: _when(s < HQ - 1, lambda: f(p)))
                    elif is_v and 2 * i + t >= 8 - late and not isinstance(s, int):
                        seq.append(functools.partial(b_desc, s, is_v, b, 2 * i + t, jnp.where(s == HQ - 1, S_T + 1, sem)))
                    else:
                        seq.append(functools.partial(b_desc, s, is_v, b, 2 * i + t, sem))
            return seq

        def issue(seq, lo, hi):
            for n in range(lo, min(hi, len(seq))):
                seq[n](n % 2)

        def rows(b, n=1):
            return pl.ds(_aligned(b * SQ, 16), n * SQ)

        def softmax_unit(q, k, p_ref, l_ref, i):
            s = lax.dot_general(q, k, NT, preferred_element_type=F32)
            p = jnp.exp2(s - jnp.max(s, axis=-1, keepdims=True))
            p_ref[i] = p.astype(BF)
            l_ref[i] = jnp.broadcast_to(1.0 / jnp.sum(p, axis=-1, keepdims=True), l_ref.shape[1:])

        def pv_unit(v, p_ref, l_ref, i):
            return (jnp.dot(p_ref[i], v, preferred_element_type=F32) * l_ref[i]).astype(BF)

        def a_qk(sl, i):
            if do_compute and "aqk" not in off:
                softmax_unit(q_v[0, rows(REP * i, REP), :], kv_v[sl, NB + i], pa_v, la_v, i)

        def a_pv(sl, i):
            if do_compute and "apv" not in off:
                o_v[0, rows(REP * i, REP), :] = pv_unit(kv_v[sl, NB + i], pa_v, la_v, i)

        def b_qk(sl, b):
            if do_compute and "bqk" not in off:
                softmax_unit(q_v[1, rows(b), :], kv_v[sl, slab(b)], pb_v, lb_v, b)

        def b_pv(sl, b):
            if do_compute and "bpv" not in off:
                o_v[1, rows(b), :] = pv_unit(kv_v[sl, slab(b)], pb_v, lb_v, b)

        def q_proj_a(a):
            if do_compute and "qp" not in off:
                q = jnp.dot(x_v[0, rows(NA * _mod(a, REP), NA), :], wq_v[0, :, gcols(_div(a, REP))], preferred_element_type=F32)
                q = (q * QSCALE).astype(BF)
                for i in range(NA):
                    for j in range(REP):
                        q_v[0, rows(REP * i + j), :] = q[i * SQ:(i + 1) * SQ, j * DH:(j + 1) * DH]

        def q_proj_b(s):
            if do_compute and "qp" not in off:
                c = pl.ds(_aligned(s * DH, DH), DH)
                q = jnp.dot(x_v[1], wq_v[1, :, c], preferred_element_type=F32)
                q_v[1] = (q * QSCALE).astype(BF)

        def o_proj_a(a):
            if do_compute and "op" not in off:
                o = jnp.concatenate(
                    [jnp.concatenate([o_v[0, rows(REP * i + j), :] for j in range(REP)], axis=1) for i in range(NA)],
                    axis=0)
                acc_v[0, rows(NA * _mod(a, REP), NA), :] += jnp.dot(o, wo_v[0, gcols(_div(a, REP)), :], preferred_element_type=F32)

        def o_proj_b(s):
            if do_compute and "op" not in off:
                r = pl.ds(_aligned(s * DH, DH), DH)
                acc_v[1] += jnp.dot(o_v[1], wo_v[1, r, :], preferred_element_type=F32)

        def phase(b_unit, a_unit, proj_a, proj_b, sl, seq):
            n = len(seq) // 2
            per = -(-n // 4)
            per += per % 2
            cut = [0, per, 2 * per, 3 * per, n] if spread is None or n != 44 else [0] + list(spread) + [n]
            for i in range(2):
                for u in range(4):
                    issue(seq, i * n + cut[u], i * n + min(cut[u + 1], n))
                    if u == apos and a_unit is not None:
                        a_unit(sl, i)
                    if u == ppos:
                        (proj_a, proj_b)[i]()
                    b_unit(sl, 4 * i + u)

        wq_perm = (lambda n: _mod(n, 8) * 8 + _div(n, 8)) if wqo == 1 else (lambda n: n)
        wo_perm = (lambda m: (m // 16) * 16 + (m % 4) * 4 + (m % 16) // 4) if woo == 1 else (lambda m: m)

        def step(s, _):
            def wq_w(i):
                return lambda br, p: _when(s < 14, lambda: wq_desc(br, 1, wq_perm(8 + 4 * s + i), p))

            def wo_w(i):
                return lambda br, p: _when(s < 27, lambda: wo_desc(br, wo_perm(20 + 4 * s + i), p))

            with scope("step"):
                sl = slot_of(s, 0)
                g = _div(s, REP)
                _when(_mod(s, REP) == 0, lambda: wait_all(wo_v.at[:, gcols(g), :], S_WO + _mod(g, 2)))
                wait_all(kv_v.at[sl], S_KV + sl)
                phase(b_qk, a_qk, functools.partial(o_proj_a, s), functools.partial(o_proj_b, jnp.maximum(s - 1, 0)), sl,
                      [d for i in range(4) for d in quad(s + 1, 0, i, wq_w(i))])
                _when(s == 14, lambda: wait_all(wq_v.at[:, :, pl.ds(2048, 2048)], S_WQ + 1))
                sl = slot_of(s, 1)
                wait_all(kv_v.at[sl], S_KV + sl)
                phase(b_pv, a_pv, functools.partial(q_proj_a, jnp.minimum(s + 2, HQ - 1)), functools.partial(q_proj_b, s + 1), sl,
                      [d for i in range(4) for d in quad(s + 1, 1, i, wo_w(i))])

        with scope("prologue"):
            part = functools.partial
            k0 = [d for i in range(4) for d in quad(0, 0, i)]
            v0 = [d for i in range(4) for d in quad(0, 1, i)]
            a0 = [part(a_desc, 0, v, i, t, 2 + v, S_A0) for t in range(8) for v in range(2) for i in range(2)]
            xs = [part(x_desc, br, i) for i in range(12) for br in range(2)]
            st = (8, 1, 4, 16, 2, 32)[pro % 10]
            wq0 = [part(wq_desc, br, 0, (i * st) % 64 + (i * st) // 64) for i in range(64) for br in range(2)]
            if pro // 10 == 0:
                seq = _interleave(xs + wq0, k0 + a0)
            elif pro // 10 == 1:
                seq = _interleave(xs + wq0, _interleave(k0, a0))
            elif pro // 10 == 2:
                seq = _interleave(_interleave(wq0, xs), _interleave(k0, a0))
            elif pro // 10 == 3:
                seq = k0 + _interleave(_interleave(wq0, xs), a0)
            elif pro // 10 == 4:
                seq = _interleave(_interleave(wq0, xs), a0) + k0
            for n in range(warm):
                seq[n](1 if n % 8 >= warm2 else 0)
            issue(seq, warm, len(seq))
            acc_v[...] = jnp.zeros_like(acc_v)
            o_v[1] = jnp.zeros((M, DH), BF)
            w = [part(wo_desc, br, wo_perm(m)) for m in range(20) for br in range(2)]
            w += [part(wq_desc, br, 1, wq_perm(i)) for i in range(8) for br in range(2)]
            seq = _interleave(w, v0)
            issue(seq, 0, cuts[0])
            with scope("p_wait"):
                wait_all(x_v, S_X)
                wait_all(wq_v.at[:, :, pl.ds(0, 2048)], S_WQ)
                wait_all(kv_v.at[pl.ds(2, 2), pl.ds(NB, NA)], S_A0)
            q_proj_a(0)
            issue(seq, cuts[0], cuts[1])
            a_qk(2, 0)
            a_qk(2, 1)
            issue(seq, cuts[1], cuts[2])
            a_pv(3, 0)
            a_pv(3, 1)
            issue(seq, cuts[2], cuts[3])
            q_proj_b(0)
            q_proj_a(1)
            issue(seq, cuts[3], len(seq))

        lax.fori_loop(0, HQ - 1, step, None)

        with scope("tail"):
            s = HQ - 1
            ksl, vsl = slot_of(s, 0), slot_of(s, 1)
            even, odd = range(0, NB, 2), range(1, NB, 2)

            def write(br, bs):
                pr = wp[0] if br == 0 else wp[1] if bs[0] % 2 == 0 else wp[2]
                if big and br == 0:
                    c = pl.ds(0, D)
                    pltpu.make_async_copy(out_v.at[:, c], out.at[:, c], sems.at[S_OUT]).start(priority=pr)
                    return
                for n, b in enumerate(bs):
                    r, c = rows(b), pl.ds(br * D, D)
                    pltpu.make_async_copy(out_v.at[r, c], out.at[r, c], sems.at[S_OUT]).start(priority=n % 2 if pr == "alt" else pr)

            def finish(bs):
                if do_compute and "tail" not in off:
                    o = jnp.concatenate([pv_unit(kv_v[vsl, slab(b)], pb_v, lb_v, b) for b in bs], axis=0)
                    y = jnp.dot(o, wo_v[1, s * DH:(s + 1) * DH, :], preferred_element_type=F32)
                    for n, b in enumerate(bs):
                        out_v[rows(b), D:2 * D] = (acc_v[1, rows(b), :] + y[n * SQ:(n + 1) * SQ]).astype(BF)

            with scope("t_waitk"):
                wait_all(kv_v.at[ksl, pl.ds(0, NB)], S_KV + ksl)
            with scope("t_qk"):
                held = [functools.partial(b_desc, s, 1, b, t, S_T) for t in range(8) for b in even]
                held = [lambda p, f=f: f(0) for f in held]
                if hold_at == 0:
                    issue(held, 0, len(held))
                    held = []
                phase(b_qk, None, functools.partial(o_proj_a, s), functools.partial(o_proj_b, s - 1), ksl, held)
                out_v[:, 0:D] = acc_v[0].astype(BF)
            if wfirst == "before_even":
                write(0, range(NB))
            with scope("t_waite"):
                wait_all(kv_v.at[vsl, pl.ds(0, NB // 2)], S_T)
            if wfirst == "mid":
                write(0, range(NB))
            if wfirst == "mid2":
                write(0, range(4))
            with scope("t_even"):
                finish(even)
            if wfirst == "mid":
                write(1, even)
            if wfirst == "mid2":
                write(0, range(4, NB))
                write(1, even)
            if wfirst == "after_even":
                write(0, range(NB))
                write(1, even)
            with scope("t_waito"):
                wait_all(kv_v.at[vsl, pl.ds(NB // 2, NB // 2), pl.ds(0, SK - 128 * late)], S_KV + vsl)
                if wfirst == "late":
                    write(0, range(NB))
                if wfirst in ("late", "before_even"):
                    write(1, even)
                if late:
                    wait_all(kv_v.at[vsl, pl.ds(NB // 2, NB // 2), pl.ds(SK - 128 * late, 128 * late)], S_T + 1)
            with scope("t_odd"):
                for bs in ((odd,), (odd[:2], odd[2:]))[split]:
                    finish(bs)
                    write(1, bs)
            with scope("t_wout"):
                pltpu.make_async_copy(out_v, out, sems.at[S_OUT]).wait()

    VM = pltpu.VMEM
    scratch = [
        VM((2, M, D), BF),
        VM((2, D, HQ * DH), BF),
        VM((2, HQ * DH, D), BF),
        VM((4, NU, SK, DH), BF),
        VM((2, M, DH), BF),
        VM((NA, REP * SQ, SK), BF),
        VM((NA, REP * SQ, DH), F32),
        VM((NB, SQ, SK), BF),
        VM((NB, SQ, DH), F32),
        VM((2, M, DH), BF),
        VM((2, M, D), F32),
        VM((M, 2 * D), BF),
        pltpu.SemaphoreType.DMA((NSEM,)),
    ]

    @jax.jit
    def fn(A_x, A_k_cache, A_v_cache, A_wq, A_wo, B_x, B_k_cache, B_v_cache, B_wq, B_wo):
        out = pl.pallas_call(
            kernel,
            out_shape=jax.ShapeDtypeStruct((M, 2 * D), BF),
            in_specs=[pl.BlockSpec(memory_space=pl.ANY)] * 10,
            out_specs=pl.BlockSpec(memory_space=pl.ANY),
            scratch_shapes=scratch,
            compiler_params=pltpu.CompilerParams(
                vmem_limit_bytes=64 * 2**20, disable_bounds_checks=nobc,
                disable_semaphore_checks=nosem, flags=flags),
        )(A_x.reshape(M, D), A_k_cache, A_v_cache, A_wq, A_wo,
          B_x.reshape(M, D), B_k_cache, B_v_cache, B_wq, B_wo)
        return out.reshape(NB, SQ, 2 * D)

    return fn


_fn = build()


@jax.jit
def pallas_concat_heads__gqa_block_cached__mha_block_cached__near_ridge_kernel(
    A_x, A_k_cache, A_v_cache, A_wq, A_wo, B_x, B_k_cache, B_v_cache, B_wq, B_wo
):
    return _fn(A_x, A_k_cache, A_v_cache, A_wq, A_wo, B_x, B_k_cache, B_v_cache, B_wq, B_wo)
```

```python
import functools
import math

import jax
import jax.experimental.pallas as pl
import jax.experimental.pallas.tpu as pltpu
import jax.numpy as jnp
from jax import lax

NB, SQ, D = 8, 48, 512
HQ, HKV, SK, DH = 32, 8, 1024, 128
REP = HQ // HKV
M = NB * SQ
GW = REP * DH
NA = NB // REP
NU = NB + NA

KV_ROWS = 128
W_ROWS = 32
WQ_ROWS, WQ_COLS = 8, HQ * DH // 2
PIECES = SK // KV_ROWS

WQ_PRE, WQ_STEPS = 8, 14
WO_PRE, WO_STEPS = 20, 27
WO_PER_GROUP = GW // W_ROWS
LATE = 2

SEM_X, SEM_PAIR0, SEM_WQ, SEM_WO, SEM_OUT, SEM_HELD, SEM_LATE, SEM_KV = 0, 1, 2, 4, 6, 7, 8, 9
NUM_SEMS = SEM_KV + 4

Q_SCALE = DH ** -0.5 * math.log2(math.e)
CONTRACT_LAST = (((1,), (1,)), ((), ()))
BF16, F32 = jnp.bfloat16, jnp.float32


def _multiple_of(i, n):
    return i if isinstance(i, int) else pl.multiple_of(i, n)


def _mod(i, n):
    return i % n if isinstance(i, int) else jnp.bitwise_and(i, n - 1)


def _div(i, n):
    return i // n if isinstance(i, int) else lax.shift_right_logical(i, n.bit_length() - 1)


def _when(cond, fn):
    if isinstance(cond, bool):
        if cond:
            fn()
    else:
        pl.when(cond)(fn)


def _interleave(a, b):
    out, k = [], 0
    for i in range(0, len(a), 2):
        out += a[i:i + 2]
        while k < len(b) and k * len(a) < (i + 2) * len(b):
            out += b[k:k + 2]
            k += 2
    return out


def _issue(copies, lo, hi):
    for n in range(lo, min(hi, len(copies))):
        copies[n](n % 2)


def _slot(s, is_v):
    return 2 * _mod(s, 2) + is_v


def _slab(b):
    return (b % 2) * (NB // 2) + b // 2


def _rows(b, n=1):
    return pl.ds(_multiple_of(b * SQ, 16), n * SQ)


def _group(g):
    return pl.ds(_multiple_of(g * GW, GW), GW)


def _head(s):
    return pl.ds(_multiple_of(s * DH, DH), DH)


def _kernel(ax, ak, av, awq, awo, bx, bk, bv, bwq, bwo, out,
            x_v, wq_v, wo_v, kv_v, q_v, pa_v, ra_v, pb_v, rb_v, o_v, acc_v, out_v, sems):
    partial = functools.partial

    def start(src, dst, sem, queue):
        pltpu.make_async_copy(src, dst, sems.at[sem]).start(priority=queue)

    def wait(buf, sem):
        pltpu.make_async_copy(buf, buf, sems.at[sem]).wait()

    def x_copy(br, i, queue):
        r = pl.ds(i * W_ROWS, W_ROWS)
        start((ax, bx)[br].at[r], x_v.at[br, r], SEM_X, queue)

    def wq_copy(br, half, i, queue):
        i = _mod(i, 8) * 8 + _div(i, 8)
        r, c = pl.ds(_multiple_of(i * WQ_ROWS, WQ_ROWS), WQ_ROWS), pl.ds(half * WQ_COLS, WQ_COLS)
        start((awq, bwq)[br].at[r, c], wq_v.at[br, r, c], SEM_WQ + half, queue)

    def wo_copy(br, i, queue):
        r = pl.ds(_multiple_of(i * W_ROWS, W_ROWS), W_ROWS)
        start((awo, bwo)[br].at[r], wo_v.at[br, r], SEM_WO + _mod(_div(i, WO_PER_GROUP), 2), queue)

    def b_copy(s, is_v, b, piece, sem, queue):
        r = pl.ds(piece * KV_ROWS, KV_ROWS)
        start((bk, bv)[is_v].at[b, s, r], kv_v.at[_slot(s, is_v), _slab(b), r], sem, queue)

    def a_copy(a, is_v, i, piece, slot, sem, queue):
        r = pl.ds(piece * KV_ROWS, KV_ROWS)
        src = (ak, av)[is_v].at[NA * _mod(a, REP) + i, _div(a, REP), r]
        start(src, kv_v.at[slot, NB + i, r], sem, queue)

    def kv_copies(s, is_v, weights=None):
        slot = _slot(s, is_v)
        copies = []
        for piece in range(PIECES):
            copies += [partial(b_copy, s, is_v, b, piece, SEM_KV + slot) for b in range(NB)]
            copies += [partial(a_copy, s + 1, is_v, i, piece, slot, SEM_KV + slot) for i in range(NA)]
            if weights is not None and piece % 2 == 1:
                copies += [partial(weights, piece // 2, br) for br in range(2)]
        return copies

    def softmax_unit(q, k, p_ref, r_ref, i):
        s = lax.dot_general(q, k, CONTRACT_LAST, preferred_element_type=F32)
        p = jnp.exp2(s - jnp.max(s, axis=-1, keepdims=True))
        p_ref[i] = p.astype(BF16)
        r_ref[i] = jnp.broadcast_to(1.0 / jnp.sum(p, axis=-1, keepdims=True), r_ref.shape[1:])

    def pv_unit(v, p_ref, r_ref, i):
        return (jnp.dot(p_ref[i], v, preferred_element_type=F32) * r_ref[i]).astype(BF16)

    def a_qk(slot, i):
        softmax_unit(q_v[0, _rows(REP * i, REP), :], kv_v[slot, NB + i], pa_v, ra_v, i)

    def a_pv(slot, i):
        o_v[0, _rows(REP * i, REP), :] = pv_unit(kv_v[slot, NB + i], pa_v, ra_v, i)

    def b_qk(slot, b):
        softmax_unit(q_v[1, _rows(b), :], kv_v[slot, _slab(b)], pb_v, rb_v, b)

    def b_pv(slot, b):
        o_v[1, _rows(b), :] = pv_unit(kv_v[slot, _slab(b)], pb_v, rb_v, b)

    def a_q_proj(a):
        x = x_v[0, _rows(NA * _mod(a, REP), NA), :]
        q = jnp.dot(x, wq_v[0, :, _group(_div(a, REP))], preferred_element_type=F32)
        q = (q * Q_SCALE).astype(BF16)
        for i in range(NA):
            for j in range(REP):
                q_v[0, _rows(REP * i + j), :] = q[i * SQ:(i + 1) * SQ, j * DH:(j + 1) * DH]

    def b_q_proj(s):
        q = jnp.dot(x_v[1], wq_v[1, :, _head(s)], preferred_element_type=F32)
        q_v[1] = (q * Q_SCALE).astype(BF16)

    def a_o_proj(a):
        o = jnp.concatenate([
            jnp.concatenate([o_v[0, _rows(REP * i + j), :] for j in range(REP)], axis=1)
            for i in range(NA)], axis=0)
        acc_v[0, _rows(NA * _mod(a, REP), NA), :] += jnp.dot(
            o, wo_v[0, _group(_div(a, REP)), :], preferred_element_type=F32)

    def b_o_proj(s):
        acc_v[1] += jnp.dot(o_v[1], wo_v[1, _head(s), :], preferred_element_type=F32)

    def phase(b_unit, a_unit, projections, slot, copies):
        n = len(copies) // 2
        chunk = 2 * pl.cdiv(n, 8)
        for i in range(2):
            for u in range(4):
                _issue(copies, i * n + u * chunk, i * n + min((u + 1) * chunk, n))
                if u == 0 and a_unit is not None:
                    a_unit(slot, i)
                if u == 1 and projections[i] is not None:
                    projections[i]()
                b_unit(slot, 4 * i + u)

    w = [partial(x_copy, br, i) for i in range(M // W_ROWS) for br in range(2)]
    w += [partial(wq_copy, br, 0, i) for i in range(D // WQ_ROWS) for br in range(2)]
    kv = kv_copies(0, 0)
    kv += [partial(a_copy, 0, is_v, i, piece, _slot(1, is_v), SEM_PAIR0)
           for piece in range(PIECES) for is_v in range(2) for i in range(NA)]
    copies = _interleave(w, kv)
    _issue(copies, 0, len(copies))
    acc_v[...] = jnp.zeros_like(acc_v)
    o_v[1] = jnp.zeros((M, DH), BF16)

    w = [partial(wo_copy, br, i) for i in range(WO_PRE) for br in range(2)]
    w += [partial(wq_copy, br, 1, i) for i in range(WQ_PRE) for br in range(2)]
    copies = _interleave(w, kv_copies(0, 1))
    _issue(copies, 0, 72)
    wait(x_v, SEM_X)
    wait(wq_v.at[:, :, pl.ds(0, WQ_COLS)], SEM_WQ)
    wait(kv_v.at[pl.ds(_slot(1, 0), 2), pl.ds(NB, NA)], SEM_PAIR0)
    a_q_proj(0)
    _issue(copies, 72, 84)
    for i in range(NA):
        a_qk(_slot(1, 0), i)
    _issue(copies, 84, 100)
    for i in range(NA):
        a_pv(_slot(1, 1), i)
    _issue(copies, 100, 116)
    b_q_proj(0)
    a_q_proj(1)
    _issue(copies, 116, len(copies))

    def step(s, carry):
        def wq_next(j, br, queue):
            _when(s < WQ_STEPS, lambda: wq_copy(br, 1, WQ_PRE + 4 * s + j, queue))

        def wo_next(j, br, queue):
            _when(s < WO_STEPS, lambda: wo_copy(br, WO_PRE + 4 * s + j, queue))

        g = _div(s, REP)
        _when(_mod(s, REP) == 0, lambda: wait(wo_v.at[:, _group(g), :], SEM_WO + _mod(g, 2)))
        slot = _slot(s, 0)
        wait(kv_v.at[slot], SEM_KV + slot)
        phase(b_qk, a_qk, (partial(a_o_proj, s), partial(b_o_proj, jnp.maximum(s - 1, 0))),
              slot, kv_copies(s + 1, 0, wq_next))
        _when(s == WQ_STEPS, lambda: wait(wq_v.at[:, :, pl.ds(WQ_COLS, WQ_COLS)], SEM_WQ + 1))
        slot = _slot(s, 1)
        wait(kv_v.at[slot], SEM_KV + slot)
        phase(b_pv, a_pv, (partial(a_q_proj, s + 2), partial(b_q_proj, s + 1)),
              slot, kv_copies(s + 1, 1, wo_next))
        return carry

    lax.fori_loop(0, HQ - 2, step, None)

    s, last = HQ - 2, HQ - 1
    k_last, v_last = _slot(last, 0), _slot(last, 1)
    even, odd = range(0, NB, 2), range(1, NB, 2)
    slot = _slot(s, 0)
    wait(kv_v.at[slot], SEM_KV + slot)
    phase(b_qk, a_qk, (partial(a_o_proj, s), partial(b_o_proj, s - 1)), slot,
          [partial(b_copy, last, 0, b, piece, SEM_KV + k_last)
           for piece in range(PIECES) for b in range(NB)])
    slot = _slot(s, 1)
    wait(kv_v.at[slot], SEM_KV + slot)
    phase(b_pv, a_pv, (None, partial(b_q_proj, last)), slot,
          [partial(b_copy, last, 1, b, piece, SEM_KV + v_last if piece < PIECES - LATE else SEM_LATE)
           if b in odd else (lambda queue: None)
           for piece in range(PIECES) for b in range(NB)])

    def finish(batches):
        o = jnp.concatenate([pv_unit(kv_v[v_last, _slab(b)], pb_v, rb_v, b) for b in batches], axis=0)
        y = jnp.dot(o, wo_v[1, _head(last), :], preferred_element_type=F32)
        for n, b in enumerate(batches):
            out_v[_rows(b), D:] = (acc_v[1, _rows(b), :] + y[n * SQ:(n + 1) * SQ]).astype(BF16)

    def write(br, batches):
        for n, b in enumerate(batches):
            r, c = _rows(b), pl.ds(br * D, D)
            start(out_v.at[r, c], out.at[r, c], SEM_OUT, n % 2)

    wait(kv_v.at[k_last, pl.ds(0, NB)], SEM_KV + k_last)
    for piece in range(PIECES):
        for b in even:
            b_copy(last, 1, b, piece, SEM_HELD, 0)
    phase(b_qk, None, (partial(a_o_proj, last), partial(b_o_proj, last - 1)), k_last, [])
    out_v[:, :D] = acc_v[0].astype(BF16)
    wait(kv_v.at[v_last, pl.ds(0, NB // 2)], SEM_HELD)
    finish(even)
    early = (PIECES - LATE) * KV_ROWS
    wait(kv_v.at[v_last, pl.ds(NB // 2, NB // 2), pl.ds(0, early)], SEM_KV + v_last)
    write(0, range(NB))
    write(1, even)
    wait(kv_v.at[v_last, pl.ds(NB // 2, NB // 2), pl.ds(early, SK - early)], SEM_LATE)
    finish(odd)
    write(1, odd)
    pltpu.make_async_copy(out_v, out, sems.at[SEM_OUT]).wait()


@jax.jit
def pallas_concat_heads__gqa_block_cached__mha_block_cached__near_ridge_kernel(
    A_x: jax.Array,
    A_k_cache: jax.Array,
    A_v_cache: jax.Array,
    A_wq: jax.Array,
    A_wo: jax.Array,
    B_x: jax.Array,
    B_k_cache: jax.Array,
    B_v_cache: jax.Array,
    B_wq: jax.Array,
    B_wo: jax.Array,
):
    vmem = pltpu.VMEM
    out = pl.pallas_call(
        _kernel,
        out_shape=jax.ShapeDtypeStruct((M, 2 * D), BF16),
        in_specs=[pl.BlockSpec(memory_space=pl.ANY)] * 10,
        out_specs=pl.BlockSpec(memory_space=pl.ANY),
        scratch_shapes=[
            vmem((2, M, D), BF16),
            vmem((2, D, HQ * DH), BF16),
            vmem((2, HQ * DH, D), BF16),
            vmem((4, NU, SK, DH), BF16),
            vmem((2, M, DH), BF16),
            vmem((NA, REP * SQ, SK), BF16),
            vmem((NA, REP * SQ, DH), F32),
            vmem((NB, SQ, SK), BF16),
            vmem((NB, SQ, DH), F32),
            vmem((2, M, DH), BF16),
            vmem((2, M, D), F32),
            vmem((M, 2 * D), BF16),
            pltpu.SemaphoreType.DMA((NUM_SEMS,)),
        ],
        compiler_params=pltpu.CompilerParams(
            vmem_limit_bytes=64 * 1024 * 1024,
            disable_semaphore_checks=True,
        ),
    )(A_x.reshape(M, D), A_k_cache, A_v_cache, A_wq, A_wo,
      B_x.reshape(M, D), B_k_cache, B_v_cache, B_wq, B_wo)
    return out.reshape(NB, SQ, 2 * D)
```

```python
import functools
import math

import jax
import jax.experimental.pallas as pl
import jax.experimental.pallas.tpu as pltpu
import jax.numpy as jnp
from jax import lax

NB, SQ, D = 8, 48, 512
HQ, HKV, SK, DH = 32, 8, 1024, 128
REP = HQ // HKV
M = NB * SQ
GW = REP * DH
NA = NB // REP
NU = NB + NA

KV_ROWS = 128
W_ROWS = 32
WQ_ROWS, WQ_COLS = 8, HQ * DH // 2
PIECES = SK // KV_ROWS

WQ_PRE, WQ_STEPS = 8, 14
WO_PRE, WO_STEPS = 20, 27
WO_PER_GROUP = GW // W_ROWS
LATE = 2

SEM_X, SEM_PAIR0, SEM_WQ, SEM_WO, SEM_KV, NUM_SEMS = 0, 1, 2, 3, 5, 7
SEM_HELD, SEM_LATE, SEM_OUT = SEM_X, SEM_PAIR0, SEM_WQ

Q_SCALE = DH ** -0.5 * math.log2(math.e)
CONTRACT_LAST = (((1,), (1,)), ((), ()))
BF16, F32 = jnp.bfloat16, jnp.float32


def _multiple_of(i, n):
    return i if isinstance(i, int) else pl.multiple_of(i, n)


def _mod(i, n):
    return i % n if isinstance(i, int) else jnp.bitwise_and(i, n - 1)


def _div(i, n):
    return i // n if isinstance(i, int) else lax.shift_right_logical(i, n.bit_length() - 1)


def _when(cond, fn):
    if isinstance(cond, bool):
        if cond:
            fn()
    else:
        pl.when(cond)(fn)


def _interleave(a, b):
    out, k = [], 0
    for i in range(0, len(a), 2):
        out += a[i:i + 2]
        while k < len(b) and k * len(a) < (i + 2) * len(b):
            out += b[k:k + 2]
            k += 2
    return out


def _issue(copies, lo, hi):
    for n in range(lo, min(hi, len(copies))):
        copies[n](n % 2)


def _slot(s, is_v):
    return 2 * _mod(s, 2) + is_v


def _slab(b):
    return (b % 2) * (NB // 2) + b // 2


def _rows(b, n=1):
    return pl.ds(_multiple_of(b * SQ, 16), n * SQ)


def _group(g):
    return pl.ds(_multiple_of(g * GW, GW), GW)


def _head(s):
    return pl.ds(_multiple_of(s * DH, DH), DH)


def _kernel(ax, ak, av, awq, awo, bx, bk, bv, bwq, bwo, out,
            x_v, wq_v, wo_v, kv_v, q_v, pa_v, ra_v, pb_v, rb_v, o_v, acc_v, out_v, sems):
    partial = functools.partial

    def start(src, dst, sem, queue):
        pltpu.make_async_copy(src, dst, sems.at[sem]).start(priority=queue)

    def wait(buf, sem):
        pltpu.make_async_copy(buf, buf, sems.at[sem]).wait()

    def x_copy(br, i, queue):
        r = pl.ds(i * W_ROWS, W_ROWS)
        start((ax, bx)[br].at[r], x_v.at[br, r], SEM_X, queue)

    def wq_copy(br, half, i, queue):
        i = _mod(i, 8) * 8 + _div(i, 8)
        r, c = pl.ds(_multiple_of(i * WQ_ROWS, WQ_ROWS), WQ_ROWS), pl.ds(half * WQ_COLS, WQ_COLS)
        start((awq, bwq)[br].at[r, c], wq_v.at[half, br, r], SEM_WQ, queue)

    def wo_copy(br, i, queue):
        g = _div(i, WO_PER_GROUP)
        src = (awo, bwo)[br].at[pl.ds(_multiple_of(i * W_ROWS, W_ROWS), W_ROWS)]
        r = pl.ds(_multiple_of(_mod(i, WO_PER_GROUP) * W_ROWS, W_ROWS), W_ROWS)
        start(src, wo_v.at[g, br, r], SEM_WO + _mod(g, 2), queue)

    def b_copy(s, is_v, b, piece, sem, queue):
        r = pl.ds(piece * KV_ROWS, KV_ROWS)
        start((bk, bv)[is_v].at[b, s, r], kv_v.at[_slot(s, is_v), _slab(b), r], sem, queue)

    def a_copy(a, is_v, i, piece, slot, sem, queue):
        r = pl.ds(piece * KV_ROWS, KV_ROWS)
        src = (ak, av)[is_v].at[NA * _mod(a, REP) + i, _div(a, REP), r]
        start(src, kv_v.at[slot, NB + i, r], sem, queue)

    def kv_copies(s, is_v, weights=None):
        slot = _slot(s, is_v)
        copies = []
        for piece in range(PIECES):
            copies += [partial(b_copy, s, is_v, b, piece, SEM_KV + is_v) for b in range(NB)]
            copies += [partial(a_copy, s + 1, is_v, i, piece, slot, SEM_KV + is_v) for i in range(NA)]
            if weights is not None and piece % 2 == 1:
                copies += [partial(weights, piece // 2, br) for br in range(2)]
        return copies

    def softmax_unit(q, k, p_ref, r_ref, i):
        s = lax.dot_general(q, k, CONTRACT_LAST, preferred_element_type=F32)
        p = jnp.exp2(s - jnp.max(s, axis=-1, keepdims=True))
        p_ref[i] = p.astype(BF16)
        r_ref[i] = jnp.broadcast_to(1.0 / jnp.sum(p, axis=-1, keepdims=True), r_ref.shape[1:])

    def pv_unit(v, p_ref, r_ref, i):
        return (jnp.dot(p_ref[i], v, preferred_element_type=F32) * r_ref[i]).astype(BF16)

    def a_qk(slot, i):
        softmax_unit(q_v[0, _rows(REP * i, REP), :], kv_v[slot, NB + i], pa_v, ra_v, i)

    def a_pv(slot, i):
        o_v[0, _rows(REP * i, REP), :] = pv_unit(kv_v[slot, NB + i], pa_v, ra_v, i)

    def b_qk(slot, b):
        softmax_unit(q_v[1, _rows(b), :], kv_v[slot, _slab(b)], pb_v, rb_v, b)

    def b_pv(slot, b):
        o_v[1, _rows(b), :] = pv_unit(kv_v[slot, _slab(b)], pb_v, rb_v, b)

    def a_q_proj(a):
        x = x_v[0, _rows(NA * _mod(a, REP), NA), :]
        g = _div(a, REP)
        w = wq_v[_div(g, HKV // 2), 0, :, _group(_mod(g, HKV // 2))]
        q = jnp.dot(x, w, preferred_element_type=F32)
        q = (q * Q_SCALE).astype(BF16)
        for i in range(NA):
            for j in range(REP):
                q_v[0, _rows(REP * i + j), :] = q[i * SQ:(i + 1) * SQ, j * DH:(j + 1) * DH]

    def b_q_proj(s):
        w = wq_v[_div(s, HQ // 2), 1, :, _head(_mod(s, HQ // 2))]
        q = jnp.dot(x_v[1], w, preferred_element_type=F32)
        q_v[1] = (q * Q_SCALE).astype(BF16)

    def a_o_proj(a):
        o = jnp.concatenate([
            jnp.concatenate([o_v[0, _rows(REP * i + j), :] for j in range(REP)], axis=1)
            for i in range(NA)], axis=0)
        acc_v[0, _rows(NA * _mod(a, REP), NA), :] += jnp.dot(
            o, wo_v[_div(a, REP), 0], preferred_element_type=F32)

    def b_wo(s):
        return wo_v[_div(s, REP), 1, _head(_mod(s, REP)), :]

    def b_o_proj(s):
        acc_v[1] += jnp.dot(o_v[1], b_wo(s), preferred_element_type=F32)

    def phase(b_unit, a_unit, projections, slot, copies):
        n = len(copies) // 2
        chunk = 2 * pl.cdiv(n, 8)
        for i in range(2):
            for u in range(4):
                _issue(copies, i * n + u * chunk, i * n + min((u + 1) * chunk, n))
                if u == 0 and a_unit is not None:
                    a_unit(slot, i)
                if u == 1 and projections[i] is not None:
                    projections[i]()
                b_unit(slot, 4 * i + u)

    w = [partial(x_copy, br, i) for i in range(M // W_ROWS) for br in range(2)]
    w += [partial(wq_copy, br, 0, i) for i in range(D // WQ_ROWS) for br in range(2)]
    kv = kv_copies(0, 0)
    kv += [partial(a_copy, 0, is_v, i, piece, _slot(1, is_v), SEM_PAIR0)
           for piece in range(PIECES) for is_v in range(2) for i in range(NA)]
    copies = _interleave(w, kv)
    _issue(copies, 0, len(copies))
    acc_v[...] = jnp.zeros_like(acc_v)
    o_v[1] = jnp.zeros((M, DH), BF16)

    w = [partial(wo_copy, br, i) for i in range(WO_PRE) for br in range(2)]
    w += [partial(wq_copy, br, 1, i) for i in range(WQ_PRE) for br in range(2)]
    copies = _interleave(w, kv_copies(0, 1))
    _issue(copies, 0, 72)
    wait(x_v, SEM_X)
    wait(wq_v.at[0], SEM_WQ)
    wait(kv_v.at[pl.ds(_slot(1, 0), 2), pl.ds(NB, NA)], SEM_PAIR0)
    a_q_proj(0)
    _issue(copies, 72, 84)
    for i in range(NA):
        a_qk(_slot(1, 0), i)
    _issue(copies, 84, 100)
    for i in range(NA):
        a_pv(_slot(1, 1), i)
    _issue(copies, 100, 116)
    b_q_proj(0)
    a_q_proj(1)
    _issue(copies, 116, len(copies))

    def step(s, carry):
        def wq_next(j, br, queue):
            _when(s < WQ_STEPS, lambda: wq_copy(br, 1, WQ_PRE + 4 * s + j, queue))

        def wo_next(j, br, queue):
            _when(s < WO_STEPS, lambda: wo_copy(br, WO_PRE + 4 * s + j, queue))

        g = _div(s, REP)
        _when(_mod(s, REP) == 0, lambda: wait(wo_v.at[g], SEM_WO + _mod(g, 2)))
        slot = _slot(s, 0)
        wait(kv_v.at[slot], SEM_KV)
        phase(b_qk, a_qk, (partial(a_o_proj, s), partial(b_o_proj, jnp.maximum(s - 1, 0))),
              slot, kv_copies(s + 1, 0, wq_next))
        _when(s == WQ_STEPS, lambda: wait(wq_v.at[1], SEM_WQ))
        slot = _slot(s, 1)
        wait(kv_v.at[slot], SEM_KV + 1)
        phase(b_pv, a_pv, (partial(a_q_proj, s + 2), partial(b_q_proj, s + 1)),
              slot, kv_copies(s + 1, 1, wo_next))
        return carry

    lax.fori_loop(0, HQ - 2, step, None)

    s, last = HQ - 2, HQ - 1
    k_last, v_last = _slot(last, 0), _slot(last, 1)
    even, odd = range(0, NB, 2), range(1, NB, 2)
    slot = _slot(s, 0)
    wait(kv_v.at[slot], SEM_KV)
    phase(b_qk, a_qk, (partial(a_o_proj, s), partial(b_o_proj, s - 1)), slot,
          [partial(b_copy, last, 0, b, piece, SEM_KV)
           for piece in range(PIECES) for b in range(NB)])
    slot = _slot(s, 1)
    wait(kv_v.at[slot], SEM_KV + 1)
    phase(b_pv, a_pv, (None, partial(b_q_proj, last)), slot,
          [partial(b_copy, last, 1, b, piece, SEM_KV + 1 if piece < PIECES - LATE else SEM_LATE)
           if b in odd else (lambda queue: None)
           for piece in range(PIECES) for b in range(NB)])

    def finish(batches):
        o = jnp.concatenate([pv_unit(kv_v[v_last, _slab(b)], pb_v, rb_v, b) for b in batches], axis=0)
        y = jnp.dot(o, b_wo(last), preferred_element_type=F32)
        for n, b in enumerate(batches):
            out_v[1, _rows(b), :] = (acc_v[1, _rows(b), :] + y[n * SQ:(n + 1) * SQ]).astype(BF16)

    def write(br, batches):
        for n, b in enumerate(batches):
            start(out_v.at[br, _rows(b)], out.at[_rows(b), pl.ds(br * D, D)], SEM_OUT, n % 2)

    wait(kv_v.at[k_last, pl.ds(0, NB)], SEM_KV)
    for piece in range(PIECES):
        for b in even:
            b_copy(last, 1, b, piece, SEM_HELD, 0)
    phase(b_qk, None, (partial(a_o_proj, last), partial(b_o_proj, last - 1)), k_last, [])
    out_v[0] = acc_v[0].astype(BF16)
    wait(kv_v.at[v_last, pl.ds(0, NB // 2)], SEM_HELD)
    finish(even)
    early = (PIECES - LATE) * KV_ROWS
    wait(kv_v.at[v_last, pl.ds(NB // 2, NB // 2), pl.ds(0, early)], SEM_KV + 1)
    write(0, range(NB))
    write(1, even)
    wait(kv_v.at[v_last, pl.ds(NB // 2, NB // 2), pl.ds(early, SK - early)], SEM_LATE)
    finish(odd)
    write(1, odd)
    wait(out, SEM_OUT)


@jax.jit
def pallas_concat_heads__gqa_block_cached__mha_block_cached__near_ridge_kernel(
    A_x: jax.Array,
    A_k_cache: jax.Array,
    A_v_cache: jax.Array,
    A_wq: jax.Array,
    A_wo: jax.Array,
    B_x: jax.Array,
    B_k_cache: jax.Array,
    B_v_cache: jax.Array,
    B_wq: jax.Array,
    B_wo: jax.Array,
):
    vmem = pltpu.VMEM
    out = pl.pallas_call(
        _kernel,
        out_shape=jax.ShapeDtypeStruct((M, 2 * D), BF16),
        in_specs=[pl.BlockSpec(memory_space=pl.ANY)] * 10,
        out_specs=pl.BlockSpec(memory_space=pl.ANY),
        scratch_shapes=[
            vmem((2, M, D), BF16),
            vmem((2, 2, D, WQ_COLS), BF16),
            vmem((HKV, 2, GW, D), BF16),
            vmem((4, NU, SK, DH), BF16),
            vmem((2, M, DH), BF16),
            vmem((NA, REP * SQ, SK), BF16),
            vmem((NA, REP * SQ, DH), F32),
            vmem((NB, SQ, SK), BF16),
            vmem((NB, SQ, DH), F32),
            vmem((2, M, DH), BF16),
            vmem((2, M, D), F32),
            vmem((2, M, D), BF16),
            pltpu.SemaphoreType.DMA((NUM_SEMS,)),
        ],
        compiler_params=pltpu.CompilerParams(vmem_limit_bytes=64 * 1024 * 1024),
    )(A_x.reshape(M, D), A_k_cache, A_v_cache, A_wq, A_wo,
      B_x.reshape(M, D), B_k_cache, B_v_cache, B_wq, B_wo)
    return out.reshape(NB, SQ, 2 * D)
```
